```python
import os as _os
_os.environ.setdefault("JAX_PLATFORMS", "cpu")
import jax
import jax.numpy as jnp

def _softmax(x, axis=-1):
    return jax.nn.softmax(x, axis=axis)
def _gelu(x):
    return jax.nn.gelu(x, approximate=True)
def _silu(x):
    return jax.nn.silu(x)
def _sigmoid(x):
    return jax.nn.sigmoid(x)
def _layernorm(x, axis=-1, eps=1e-5):
    m = jnp.mean(x, axis=axis, keepdims=True)
    v = jnp.var(x, axis=axis, keepdims=True)
    return (x - m) / jnp.sqrt(v + eps)
def _scatter_add(tgt, idx, src, axis=0):
    return tgt.at[idx].add(src)
def _segment_sum(src, seg, n):
    return jax.ops.segment_sum(src, seg, n)
class _Rng:
    def __init__(self, key):
        self._k = key
    def _next(self):
        self._k, sub = jax.random.split(self._k)
        return sub
    def normal(self, shape):
        return jax.random.normal(self._next(), shape, dtype=jnp.bfloat16)
    def randint(self, lo, hi, shape):
        return jax.random.randint(self._next(), shape, lo, hi, dtype=jnp.int32)
    def uniform(self, shape, lo=0.0, hi=1.0):
        return jax.random.uniform(self._next(), shape, jnp.bfloat16, lo, hi)
    def permutation(self, n):
        return jax.random.permutation(self._next(), n)


kernel_name = 'concat_heads__compressed_kv_cla__compressed_kv_cla__decode'

def setup_inputs():
    _rng = _Rng(jax.random.key(int.from_bytes(__import__("os").urandom(4), "little")))
    _w = (lambda a: (lambda t: t.astype(jnp.bfloat16) if jnp.issubdtype(t.dtype, jnp.floating) else t)(jnp.asarray(a)))
    def _A_setup():
        B, H, Sq, Sk, D, M = 4, 32, 1, 4096, 128, 640
        Dc = 4 * D
        return {
            "x": _w((lambda *s: _rng.normal(s) * 1.6)(B, Sq, M)),
            "c_kv": _w((lambda *s: _rng.normal(s) * 0.05)(B, Sk, Dc)),
            "w_q": _w((lambda *s: _rng.normal(s) * 1.6)(M, H, D) * (M ** -0.5)),
            "w_uk": _w((lambda *s: _rng.normal(s) * 1.6)(Dc, H, D) * (Dc ** -0.5)),
            "w_uv": _w((lambda *s: _rng.normal(s) * 0.05)(Dc, H, D) * (Dc ** -0.5)),
            "w_o": _w((lambda *s: _rng.normal(s) * 0.05)(H, D, M) * ((H * D) ** -0.5)),
        }
    _A_in = _A_setup()

    def _B_setup():
        B, H, Sq, Sk, D, M = 4, 32, 1, 4096, 128, 640
        Dc = 4 * D
        return {
            "x": _w((lambda *s: _rng.normal(s) * 1.6)(B, Sq, M)),
            "c_kv": _w((lambda *s: _rng.normal(s) * 0.05)(B, Sk, Dc)),
            "w_q": _w((lambda *s: _rng.normal(s) * 1.6)(M, H, D) * (M ** -0.5)),
            "w_uk": _w((lambda *s: _rng.normal(s) * 1.6)(Dc, H, D) * (Dc ** -0.5)),
            "w_uv": _w((lambda *s: _rng.normal(s) * 0.05)(Dc, H, D) * (Dc ** -0.5)),
            "w_o": _w((lambda *s: _rng.normal(s) * 0.05)(H, D, M) * ((H * D) ** -0.5)),
        }
    _B_in = _B_setup()

    return {
        "A_x": _A_in["x"],
        "A_c_kv": _A_in["c_kv"],
        "A_w_q": _A_in["w_q"],
        "A_w_uk": _A_in["w_uk"],
        "A_w_uv": _A_in["w_uv"],
        "A_w_o": _A_in["w_o"],
        "B_x": _B_in["x"],
        "B_c_kv": _B_in["c_kv"],
        "B_w_q": _B_in["w_q"],
        "B_w_uk": _B_in["w_uk"],
        "B_w_uv": _B_in["w_uv"],
        "B_w_o": _B_in["w_o"],
    }

def reference(A_x, A_c_kv, A_w_q, A_w_uk, A_w_uv, A_w_o, B_x, B_c_kv, B_w_q, B_w_uk, B_w_uv, B_w_o):
    def _A_ref(x, c_kv, w_q, w_uk, w_uv, w_o):
        B, Sq, M = x.shape[0], x.shape[1], x.shape[2]
        Sk = c_kv.shape[1]
        H, D = w_q.shape[1], w_q.shape[2]
        q = jnp.einsum("bqm,mhd->bhqd", x, w_q)
        k = jnp.einsum("bkc,chd->bhkd", c_kv, w_uk)
        v = jnp.einsum("bkc,chd->bhkd", c_kv, w_uv)
        scores = jnp.einsum("bhqd,bhkd->bhqk", q, k) * (D ** -0.5)
        off = Sk - Sq
        qi = jnp.arange(Sq)[:, None]
        kj = jnp.arange(Sk)[None, :]
        cmask = kj <= (qi + off)
        scores = jnp.where(cmask[None, None], scores, -1e9)
        p = _softmax(scores, axis=-1)
        ctx = jnp.einsum("bhqk,bhkd->bhqd", p, v)
        return jnp.einsum("bhqd,hdm->bqm", ctx, w_o)

    def _B_ref(x, c_kv, w_q, w_uk, w_uv, w_o):
        B, Sq, M = x.shape[0], x.shape[1], x.shape[2]
        Sk = c_kv.shape[1]
        H, D = w_q.shape[1], w_q.shape[2]
        q = jnp.einsum("bqm,mhd->bhqd", x, w_q)
        k = jnp.einsum("bkc,chd->bhkd", c_kv, w_uk)
        v = jnp.einsum("bkc,chd->bhkd", c_kv, w_uv)
        scores = jnp.einsum("bhqd,bhkd->bhqk", q, k) * (D ** -0.5)
        off = Sk - Sq
        qi = jnp.arange(Sq)[:, None]
        kj = jnp.arange(Sk)[None, :]
        cmask = kj <= (qi + off)
        scores = jnp.where(cmask[None, None], scores, -1e9)
        p = _softmax(scores, axis=-1)
        ctx = jnp.einsum("bhqk,bhkd->bhqd", p, v)
        return jnp.einsum("bhqd,hdm->bqm", ctx, w_o)

    a = _A_ref(A_x, A_c_kv, A_w_q, A_w_uk, A_w_uv, A_w_o)
    b = _B_ref(B_x, B_c_kv, B_w_q, B_w_uk, B_w_uv, B_w_o)
    return jnp.concatenate([a, b], axis=-1)
```

```python
import functools
import jax
import jax.numpy as jnp
from jax import lax
from jax.experimental import pallas as pl
from jax.experimental.pallas import tpu as pltpu

F32 = jnp.float32
BF16 = jnp.bfloat16
U32 = jnp.uint32

WO_LAST_CHUNKS = (8, 4, 2, 1, 1)
TK = 512


def _kernel(xA, ckvA, wqA, wukA, wuvA, woA, xB, ckvB, wqB, wukB, wuvB, woB,
            o_ref,
            x_s, ckv_s, wq_s, wuk_s, wuv_s, wo_s,
            q_s, o2_s, qa_s, s_s, ct_s, e3_s, cj_s, sems,
            *, B, H, SK, D, M, DC):
    NP = H // 2
    nk = SK // TK
    scale = float(D) ** -0.5
    xs = (xA, xB); ckvs = (ckvA, ckvB); wqs = (wqA, wqB); wuks = (wukA, wukB)
    wuvs = (wuvA, wuvB); wos = (woA, woB)
    NQ = M * H
    NU = DC * H
    NO = H * D

    def sem_x(br): return br
    def sem_wq(br): return 2 + 7 * br
    def sem_wuk(br): return 3 + 7 * br
    def sem_ckv(br, b): return 4 + 7 * br + b
    def sem_wuv(br): return 8 + 7 * br
    SEM_WO = 16

    for br in range(2):
        pltpu.make_async_copy(xs[br], x_s.at[br], sems.at[sem_x(br)]).start()
    for br in range(2):
        pltpu.make_async_copy(wqs[br], wq_s.at[pl.ds(br * NQ, NQ)], sems.at[sem_wq(br)]).start()
        pltpu.make_async_copy(wuks[br], wuk_s.at[pl.ds(br * NU, NU)], sems.at[sem_wuk(br)]).start()
        for b in range(B):
            pltpu.make_async_copy(ckvs[br].at[b], ckv_s.at[pl.ds((br * B + b) * SK, SK)],
                                  sems.at[sem_ckv(br, b)]).start()
        pltpu.make_async_copy(wuvs[br], wuv_s.at[pl.ds(br * NU, NU)], sems.at[sem_wuv(br)]).start()
    pltpu.make_async_copy(wos[0], wo_s.at[pl.ds(0, NO)], sems.at[SEM_WO]).start()
    r0 = 0
    wo_starts = []
    for ci, n in enumerate(WO_LAST_CHUNKS):
        wo_starts.append(r0)
        pltpu.make_async_copy(wos[1].at[pl.ds(r0 * 256, n * 256)],
                              wo_s.at[pl.ds(NO + r0 * 256, n * 256)], sems.at[SEM_WO + 1 + ci]).start()
        r0 += n
    assert r0 * 256 == NO

    def wait(buf, sem):
        pltpu.make_async_copy(buf, buf, sems.at[sem]).wait()

    ii = lax.broadcasted_iota(jnp.int32, (128, 256), 0)
    ll = lax.broadcasted_iota(jnp.int32, (128, 256), 1)
    dup = jnp.where((ll >> 1) == ii, 1.0, 0.0).astype(BF16)
    ii = lax.broadcasted_iota(jnp.int32, (256, 128), 0)
    ll = lax.broadcasted_iota(jnp.int32, (256, 128), 1)
    cmp0 = jnp.where((ii >> 1) == ll, 1.0, 0.0).astype(BF16)

    def parity_mask(rows, cols):
        r = lax.broadcasted_iota(jnp.int32, (rows, cols), 0)
        l = lax.broadcasted_iota(jnp.int32, (rows, cols), 1)
        return ((r >> 2) & 1) == (l & 1)

    wq32 = wq_s.bitcast(U32)
    wuk32 = wuk_s.bitcast(U32)
    wuv32 = wuv_s.bitcast(U32)

    def branch(br, _):
        wait(x_s.at[br], br)
        row = lax.broadcasted_iota(jnp.int32, (8, M), 0)
        x8 = jnp.zeros((8, M), F32)
        x4 = x_s[br].astype(F32)
        for b in range(B):
            xb = x4[b:b + 1, :]
            x8 = jnp.where((row & 3) == b, jnp.broadcast_to(xb, (8, M)), x8)
        x8 = x8.astype(BF16)
        pm = parity_mask(8, 256)
        xexp = jnp.concatenate(
            [jnp.where(pm, jnp.dot(x8[:, t * 128:(t + 1) * 128], dup, preferred_element_type=F32), 0.0)
             for t in range(M // 128)], axis=1).astype(BF16)

        wait(wq_s.at[pl.ds(0, NQ)], 2 + 7 * br)

        def pair_rows(w32, nrows_half, cnt, jj, r):
            off = pl.multiple_of(br * nrows_half + jj * 4, 4)
            v = w32.at[pl.ds(off, (cnt - 1) * NP + 4)]
            return pltpu.bitcast(v[pl.ds(r, cnt, stride=NP), :], BF16)

        def q_body(jj, _):
            for r in range(4):
                w = pair_rows(wq32, NQ // 2, M, jj, r)
                q_s[pl.ds(pl.multiple_of(jj * 32 + r * 8, 8), 8), :] = jnp.dot(xexp, w, preferred_element_type=F32)
            return 0
        lax.fori_loop(0, NP // 4, q_body, 0)

        wait(wuk_s.at[pl.ds(0, NU)], 3 + 7 * br)
        pm2 = parity_mask(8, 2 * DC)

        def qa_body(jj, _):
            for r in range(4):
                w = pair_rows(wuk32, NU // 2, DC, jj, r)
                rr = pl.multiple_of(jj * 32 + r * 8, 8)
                qj = q_s[pl.ds(rr, 8), :].astype(BF16)
                o = lax.dot_general(qj, w, (((1,), (1,)), ((), ())), preferred_element_type=F32)
                o2_s[pl.ds(rr, 8), :] = jnp.where(pm2, o * scale, 0.0)
            return 0
        lax.fori_loop(0, NP // 4, qa_body, 0)
        for t in range(DC // 128):
            qa_s[t] = jnp.dot(
                o2_s[:, t * 256:(t + 1) * 256].astype(BF16), cmp0, preferred_element_type=F32)

        def att(b, _):
            wait(ckv_s.at[pl.ds(0, SK)], 4 + 7 * br + b)
            qa_b = jnp.concatenate(
                [jnp.concatenate([qa_s[t, pl.ds(b, NP, stride=8), :], qa_s[t, pl.ds(4 + b, NP, stride=8), :]], axis=0)
                 for t in range(DC // 128)], axis=1).astype(BF16)
            base = (br * B + b) * SK

            def s_body(i, m):
                kc = ckv_s[pl.ds(pl.multiple_of(base + i * TK, TK), TK), :]
                s = lax.dot_general(qa_b, kc, (((1,), (1,)), ((), ())), preferred_element_type=F32)
                s_s[i] = s
                for t in range(TK // 128):
                    m = jnp.maximum(m, s[:, t * 128:(t + 1) * 128])
                return m
            m = lax.fori_loop(0, nk, s_body, jnp.full((H, 128), -jnp.inf, F32))
            m = jnp.max(m, axis=1, keepdims=True)

            def pv_body(i, carry):
                acc, l = carry
                p = jnp.exp(s_s[i] - m)
                for t in range(TK // 128):
                    l = l + p[:, t * 128:(t + 1) * 128]
                kc = ckv_s[pl.ds(pl.multiple_of(base + i * TK, TK), TK), :]
                acc = acc + jnp.dot(p.astype(BF16), kc, preferred_element_type=F32)
                return acc, l
            acc, l = lax.fori_loop(0, nk, pv_body,
                                   (jnp.zeros((H, DC), F32), jnp.zeros((H, 128), F32)))
            ctxc = acc / jnp.sum(l, axis=1, keepdims=True)
            for t in range(DC // 128):
                ct_s[t, pl.ds(b, NP, stride=8), :] = ctxc[0:NP, t * 128:(t + 1) * 128]
                ct_s[t, pl.ds(4 + b, NP, stride=8), :] = ctxc[NP:H, t * 128:(t + 1) * 128]
            return 0
        lax.fori_loop(0, B, att, 0)

        pm3 = parity_mask(128, 256)
        for t in range(DC // 128):
            e = jnp.dot(ct_s[t].astype(BF16), dup, preferred_element_type=F32)
            e3_s[:, t * 256:(t + 1) * 256] = jnp.where(pm3, e, 0.0)
        wait(wuv_s.at[pl.ds(0, NU)], 8 + 7 * br)

        def c_body(jj, _):
            for r in range(4):
                w = pair_rows(wuv32, NU // 2, DC, jj, r)
                rr = pl.multiple_of(jj * 32 + r * 8, 8)
                e = e3_s[pl.ds(rr, 8), :].astype(BF16)
                cj_s[br * NP + jj * 4 + r] = jnp.dot(e, w, preferred_element_type=F32)
            return 0
        lax.fori_loop(0, NP // 4, c_body, 0)
        return 0

    lax.fori_loop(0, 2, branch, 0)

    row8 = lax.broadcasted_iota(jnp.int32, (8, 128), 0)

    def o_body(i, acc):
        @pl.when(i == 0)
        def _():
            wait(wo_s.at[pl.ds(0, NO)], SEM_WO)
        for ci, n in enumerate(WO_LAST_CHUNKS):
            @pl.when(i == NP + wo_starts[ci])
            def _():
                wait(wo_s.at[pl.ds(0, n * 256)], SEM_WO + 1 + ci)
        cj = cj_s[i]
        lhs = jnp.concatenate([jnp.where(row8 < 4, cj, 0.0), jnp.where(row8 >= 4, cj, 0.0)],
                              axis=1).astype(BF16)
        w = wo_s[pl.ds(pl.multiple_of(i * 256, 256), 256), :]
        return acc + jnp.dot(lhs, w, preferred_element_type=F32)

    for br in range(2):
        acc = lax.fori_loop(br * NP, (br + 1) * NP, o_body, jnp.zeros((8, M), F32))
        out = (acc[0:4] + acc[4:8]).astype(BF16)
        o_ref[:, br * M:(br + 1) * M] = out


@jax.jit
def pallas_concat_heads__compressed_kv_cla__compressed_kv_cla__decode_kernel(A_x, A_c_kv, A_w_q, A_w_uk, A_w_uv, A_w_o, B_x, B_c_kv, B_w_q, B_w_uk, B_w_uv, B_w_o):
    B, _, M = A_x.shape
    SK, DC = A_c_kv.shape[1], A_c_kv.shape[2]
    H, D = A_w_q.shape[1], A_w_q.shape[2]

    def prep(x, ckv, wq, wuk, wuv, wo):
        return (x.reshape(B, M), ckv, wq.reshape(M * H, D), wuk.reshape(DC * H, D), wuv.reshape(DC * H, D),
                wo.reshape(H * D, M))
    args = prep(A_x, A_c_kv, A_w_q, A_w_uk, A_w_uv, A_w_o) + prep(B_x, B_c_kv, B_w_q, B_w_uk, B_w_uv, B_w_o)
    nsem = 17 + len(WO_LAST_CHUNKS)
    out = pl.pallas_call(
        functools.partial(_kernel, B=B, H=H, SK=SK, D=D, M=M, DC=DC),
        out_shape=jax.ShapeDtypeStruct((B, 2 * M), BF16),
        in_specs=[pl.BlockSpec(memory_space=pl.ANY)] * 12,
        out_specs=pl.BlockSpec(memory_space=pltpu.VMEM),
        scratch_shapes=[
            pltpu.VMEM((2, B, M), BF16),
            pltpu.VMEM((2 * B * SK, DC), BF16),
            pltpu.VMEM((2 * M * H, D), BF16),
            pltpu.VMEM((2 * DC * H, D), BF16),
            pltpu.VMEM((2 * DC * H, D), BF16),
            pltpu.VMEM((2 * H * D, M), BF16),
            pltpu.VMEM((128, 128), F32),
            pltpu.VMEM((128, 2 * DC), F32),
            pltpu.VMEM((DC // 128, 128, 128), F32),
            pltpu.VMEM((SK // TK, H, TK), F32),
            pltpu.VMEM((DC // 128, 128, 128), F32),
            pltpu.VMEM((128, 2 * DC), F32),
            pltpu.VMEM((H, 8, 128), F32),
            pltpu.SemaphoreType.DMA((nsem,)),
        ],
        compiler_params=pltpu.CompilerParams(vmem_limit_bytes=100 * 1024 * 1024),
    )(*args)
    return out.reshape(B, 1, 2 * M)
```

```python
import functools

import jax
import jax.numpy as jnp
from jax import lax
from jax.experimental import pallas as pl
from jax.experimental.pallas import tpu as pltpu

F32 = jnp.float32
BF16 = jnp.bfloat16
U32 = jnp.uint32

TK = 512
PITCH = 24
CB = 8
WO_LAST_CHUNKS = (16, 8, 4, 2, 1, 1)
SEM_WO = 16
SEM_OUT = SEM_WO + 1 + len(WO_LAST_CHUNKS)
N_SEMS = SEM_OUT + 2


def _body(xA, ckvA, wqA, wukA, wuvA, woA, xB, ckvB, wqB, wukB, wuvB, woB,
          o_hbm,
          x_s, ckv_s, wq_s, wuk_s, wuv_s, wo_s,
          u_s, q_s, o2_s, qa_s, s_s, ct_s, e3_s, cj_s, oa_s, ob_s, sems,
          *, B, H, SK, D, M, DC):
    NP = H // 2
    nk = SK // TK
    scale = float(D) ** -0.5
    xs = (xA, xB); ckvs = (ckvA, ckvB); wqs = (wqA, wqB); wuks = (wukA, wukB)
    wuvs = (wuvA, wuvB); wos = (woA, woB)
    NQ = M * H
    NU = DC * H
    NO = H * D

    def dst_x(br): return x_s.at[br], br
    def dst_wq(br): return wq_s.at[pl.ds(pl.multiple_of(br * NQ, NQ), NQ)], 2 + 7 * br
    def dst_wuk(br): return wuk_s.at[pl.ds(pl.multiple_of(br * NU, NU), NU)], 3 + 7 * br
    def dst_ckv(br, b): return ckv_s.at[pl.ds(pl.multiple_of((br * B + b) * SK, SK), SK)], 4 + 7 * br + b
    def dst_wuv(br): return wuv_s.at[pl.ds(pl.multiple_of(br * NU, NU), NU)], 8 + 7 * br

    def start(src, dst_sem):
        pltpu.make_async_copy(src, dst_sem[0], sems.at[dst_sem[1]]).start()

    def wait(dst_sem):
        pltpu.make_async_copy(dst_sem[0], dst_sem[0], sems.at[dst_sem[1]]).wait()

    for br in range(2):
        start(wqs[br], dst_wq(br))
        if br == 0:
            start(xs[0], dst_x(0))
            start(xs[1], dst_x(1))
        start(wuks[br], dst_wuk(br))
        for b in range(B):
            start(ckvs[br].at[b], dst_ckv(br, b))
        start(wuvs[br], dst_wuv(br))
    wo_dsts = [(wo_s.at[pl.ds(0, NO)], SEM_WO)]
    start(wos[0], wo_dsts[0])
    wo_starts = []
    h0 = 0
    for ci, n in enumerate(WO_LAST_CHUNKS):
        wo_starts.append(h0)
        wo_dsts.append((wo_s.at[pl.ds(NO + h0 * D, n * D)], SEM_WO + 1 + ci))
        start(wos[1].at[pl.ds(h0 * D, n * D)], wo_dsts[-1])
        h0 += n
    assert h0 == H

    ii = lax.broadcasted_iota(jnp.int32, (128, 256), 0)
    ll = lax.broadcasted_iota(jnp.int32, (128, 256), 1)
    dup = jnp.where((ll >> 1) == ii, 1.0, 0.0).astype(BF16)
    ii = lax.broadcasted_iota(jnp.int32, (256, 128), 0)
    ll = lax.broadcasted_iota(jnp.int32, (256, 128), 1)
    cmp0 = jnp.where((ii >> 1) == ll, 1.0, 0.0).astype(BF16)

    def parity_mask(rows, cols):
        r = lax.broadcasted_iota(jnp.int32, (rows, cols), 0)
        l = lax.broadcasted_iota(jnp.int32, (rows, cols), 1)
        return ((r >> 2) & 1) == (l & 1)

    def branch(br, _):
        def stage(w_s, cnt):
            def cp(i, _):
                src = pl.multiple_of((br * cnt + i * CB) * H, CB * H)
                v = pltpu.bitcast(w_s[pl.ds(src, CB * H), :], U32)
                blk = u_s.at[pl.ds(pl.multiple_of(i * (CB * PITCH), 8), CB * PITCH)]
                for c in range(CB):
                    blk[c * PITCH:c * PITCH + NP, :] = v[c * NP:(c + 1) * NP, :]
                return 0
            lax.fori_loop(0, cnt // CB, cp, 0)

        def pair_rows(cnt, jj, r):
            v = u_s.at[pl.ds(pl.multiple_of(jj * 8, 8), (cnt - 1) * PITCH + 8)]
            return pltpu.bitcast(v[pl.ds(r, cnt, stride=PITCH), :], BF16)

        wait(dst_x(br))
        row = lax.broadcasted_iota(jnp.int32, (8, M), 0)
        x8 = jnp.zeros((8, M), F32)
        x4 = x_s[br].astype(F32)
        for b in range(B):
            x8 = jnp.where((row & 3) == b, jnp.broadcast_to(x4[b:b + 1, :], (8, M)), x8)
        x8 = x8.astype(BF16)
        pm = parity_mask(8, 256)
        xexp = jnp.concatenate(
            [jnp.where(pm, jnp.dot(x8[:, t * 128:(t + 1) * 128], dup, preferred_element_type=F32), 0.0)
             for t in range(M // 128)], axis=1).astype(BF16)

        wait(dst_wq(br))
        stage(wq_s, M)

        def q_body(jj, _):
            for r in range(8):
                q_s[pl.ds(pl.multiple_of(jj * 64 + r * 8, 8), 8), :] = jnp.dot(
                    xexp, pair_rows(M, jj, r), preferred_element_type=F32)
            return 0
        lax.fori_loop(0, NP // 8, q_body, 0)

        wait(dst_wuk(br))
        stage(wuk_s, DC)
        pm2 = parity_mask(8, 2 * DC)

        def qa_body(jj, _):
            for r in range(8):
                rr = pl.multiple_of(jj * 64 + r * 8, 8)
                qj = q_s[pl.ds(rr, 8), :].astype(BF16)
                o = lax.dot_general(qj, pair_rows(DC, jj, r), (((1,), (1,)), ((), ())),
                                    preferred_element_type=F32)
                o2_s[pl.ds(rr, 8), :] = jnp.where(pm2, o * scale, 0.0)
            return 0
        lax.fori_loop(0, NP // 8, qa_body, 0)
        for t in range(DC // 128):
            qa_s[t] = jnp.dot(o2_s[:, t * 256:(t + 1) * 256].astype(BF16), cmp0, preferred_element_type=F32)

        def att(b, _):
            wait(dst_ckv(br, b))
            qa_b = jnp.concatenate(
                [jnp.concatenate([qa_s[t, pl.ds(b, NP, stride=8), :], qa_s[t, pl.ds(4 + b, NP, stride=8), :]], axis=0)
                 for t in range(DC // 128)], axis=1).astype(BF16)
            base = (br * B + b) * SK

            def s_body(i, m):
                kc = ckv_s[pl.ds(pl.multiple_of(base + i * TK, TK), TK), :]
                s = lax.dot_general(qa_b, kc, (((1,), (1,)), ((), ())), preferred_element_type=F32)
                s_s[i] = s
                for t in range(TK // 128):
                    m = jnp.maximum(m, s[:, t * 128:(t + 1) * 128])
                return m
            m = lax.fori_loop(0, nk, s_body, jnp.full((H, 128), -jnp.inf, F32))
            m = jnp.max(m, axis=1, keepdims=True)

            def pv_body(i, carry):
                acc, l = carry
                p = jnp.exp(s_s[i] - m)
                for t in range(TK // 128):
                    l = l + p[:, t * 128:(t + 1) * 128]
                kc = ckv_s[pl.ds(pl.multiple_of(base + i * TK, TK), TK), :]
                acc = acc + jnp.dot(p.astype(BF16), kc, preferred_element_type=F32)
                return acc, l
            acc, l = lax.fori_loop(0, nk, pv_body,
                                   (jnp.zeros((H, DC), F32), jnp.zeros((H, 128), F32)))
            cc = acc / jnp.sum(l, axis=1, keepdims=True)
            for t in range(DC // 128):
                ct_s[t, pl.ds(b, NP, stride=8), :] = cc[0:NP, t * 128:(t + 1) * 128]
                ct_s[t, pl.ds(4 + b, NP, stride=8), :] = cc[NP:H, t * 128:(t + 1) * 128]
            return 0
        lax.fori_loop(0, B, att, 0)

        pm3 = parity_mask(128, 256)
        for t in range(DC // 128):
            e = jnp.dot(ct_s[t].astype(BF16), dup, preferred_element_type=F32)
            e3_s[:, t * 256:(t + 1) * 256] = jnp.where(pm3, e, 0.0)
        wait(dst_wuv(br))
        stage(wuv_s, DC)

        def c_body(jj, _):
            for r in range(8):
                e = e3_s[pl.ds(pl.multiple_of(jj * 64 + r * 8, 8), 8), :].astype(BF16)
                cj_s[br * NP + jj * 8 + r] = jnp.dot(e, pair_rows(DC, jj, r), preferred_element_type=F32)
            return 0
        lax.fori_loop(0, NP // 8, c_body, 0)
        return 0

    lax.fori_loop(0, 2, branch, 0)

    row8 = lax.broadcasted_iota(jnp.int32, (8, D), 0)

    def o_body(i, acc):
        @pl.when(i == 0)
        def _():
            wait(wo_dsts[0])
        for ci in range(len(WO_LAST_CHUNKS) - 2):
            @pl.when(i == NP + wo_starts[ci] // 2)
            def _():
                wait(wo_dsts[1 + ci])
        cj = cj_s[i]
        lhs = jnp.concatenate([jnp.where(row8 < 4, cj, 0.0), jnp.where(row8 >= 4, cj, 0.0)],
                              axis=1).astype(BF16)
        w = wo_s[pl.ds(pl.multiple_of(i * 2 * D, 2 * D), 2 * D), :]
        return acc + jnp.dot(lhs, w, preferred_element_type=F32)

    out_a = pltpu.make_async_copy(oa_s, o_hbm.at[:, pl.ds(0, M)], sems.at[SEM_OUT])
    out_b = pltpu.make_async_copy(ob_s, o_hbm.at[:, pl.ds(M, M)], sems.at[SEM_OUT + 1])

    acc = lax.fori_loop(0, NP, o_body, jnp.zeros((8, M), F32))
    oa_s[...] = (acc[0:4] + acc[4:8]).astype(BF16)
    out_a.start()

    assert WO_LAST_CHUNKS[-2:] == (1, 1) and all(s % 2 == 0 for s in wo_starts[:-1])
    acc = lax.fori_loop(NP, 2 * NP - 1, o_body, jnp.zeros((8, M), F32))
    cj = cj_s[2 * NP - 1]
    r0 = 2 * NO - 2 * D
    pre = acc[0:4] + acc[4:8]
    lhs_a = cj[0:4].astype(BF16)
    lhs_b = cj[4:8].astype(BF16)
    out_a.wait()
    wait(wo_dsts[-2])
    pre = pre + jnp.dot(lhs_a, wo_s[r0:r0 + D, :], preferred_element_type=F32)
    wait(wo_dsts[-1])
    last = jnp.dot(lhs_b, wo_s[r0 + D:r0 + 2 * D, :], preferred_element_type=F32)
    ob_s[...] = (pre + last).astype(BF16)
    out_b.start()
    out_b.wait()


def _kernel(*refs, **dims):
    pl.run_scoped(functools.partial(_body, *refs, **dims), pltpu.SemaphoreType.DMA((N_SEMS,)))


@jax.jit
def pallas_concat_heads__compressed_kv_cla__compressed_kv_cla__decode_kernel(A_x, A_c_kv, A_w_q, A_w_uk, A_w_uv, A_w_o, B_x, B_c_kv, B_w_q, B_w_uk, B_w_uv, B_w_o):
    B, _, M = A_x.shape
    SK, DC = A_c_kv.shape[1], A_c_kv.shape[2]
    H, D = A_w_q.shape[1], A_w_q.shape[2]
    assert B == 4 and H == 32 and D == 128 and A_x.shape[1] == 1

    def prep(x, ckv, wq, wuk, wuv, wo):
        return (x.reshape(B, M), ckv, wq.reshape(M * H, D), wuk.reshape(DC * H, D), wuv.reshape(DC * H, D),
                wo.reshape(H * D, M))
    args = prep(A_x, A_c_kv, A_w_q, A_w_uk, A_w_uv, A_w_o) + prep(B_x, B_c_kv, B_w_q, B_w_uk, B_w_uv, B_w_o)
    out = pl.pallas_call(
        functools.partial(_kernel, B=B, H=H, SK=SK, D=D, M=M, DC=DC),
        out_shape=jax.ShapeDtypeStruct((B, 2 * M), BF16),
        in_specs=[pl.BlockSpec(memory_space=pl.ANY)] * 12,
        out_specs=pl.BlockSpec(memory_space=pl.ANY),
        scratch_shapes=[
            pltpu.VMEM((2, B, M), BF16),
            pltpu.VMEM((2 * B * SK, DC), BF16),
            pltpu.VMEM((2 * M * H, D), BF16),
            pltpu.VMEM((2 * DC * H, D), BF16),
            pltpu.VMEM((2 * DC * H, D), BF16),
            pltpu.VMEM((2 * H * D, M), BF16),
            pltpu.VMEM((max(M, DC) * PITCH, D), U32),
            pltpu.VMEM((128, 128), F32),
            pltpu.VMEM((128, 2 * DC), F32),
            pltpu.VMEM((DC // 128, 128, 128), F32),
            pltpu.VMEM((SK // TK, H, TK), F32),
            pltpu.VMEM((DC // 128, 128, 128), F32),
            pltpu.VMEM((128, 2 * DC), F32),
            pltpu.VMEM((H, 8, 128), F32),
            pltpu.VMEM((B, M), BF16),
            pltpu.VMEM((B, M), BF16),
        ],
        compiler_params=pltpu.CompilerParams(vmem_limit_bytes=100 * 1024 * 1024),
    )(*args)
    return out.reshape(B, 1, 2 * M)
```
